```python
import jax
import jax.numpy as jnp

def _softmax(x, axis=-1):
    return jax.nn.softmax(x, axis=axis)

def _gelu(x):
    return jax.nn.gelu(x, approximate=True)

def _silu(x):
    return jax.nn.silu(x)

def _sigmoid(x):
    return jax.nn.sigmoid(x)

def _layernorm(x, axis=-1, eps=1e-05):
    m = jnp.mean(x, axis=axis, keepdims=True)
    v = jnp.var(x, axis=axis, keepdims=True)
    return (x - m) / jnp.sqrt(v + eps)

def _scatter_add(tgt, idx, src, axis=0):
    return tgt.at[idx].add(src)

def _segment_sum(src, seg, n):
    return jax.ops.segment_sum(src, seg, n)

class _Rng:

    def __init__(self, key):
        self._k = key

    def _next(self):
        self._k, sub = jax.random.split(self._k)
        return sub

    def normal(self, shape):
        return jax.random.normal(self._next(), shape, dtype=jnp.bfloat16)

    def randint(self, lo, hi, shape):
        return jax.random.randint(self._next(), shape, lo, hi, dtype=jnp.int32)

    def uniform(self, shape, lo=0.0, hi=1.0):
        return jax.random.uniform(self._next(), shape, jnp.bfloat16, lo, hi)

    def permutation(self, n):
        return jax.random.permutation(self._next(), n)
kernel_name = 'recurrent_scan__memory_aug_recurrent_mem_tr__glu_gated_glu__prompt'

def setup_inputs():
    _rng = _Rng(jax.random.key(int.from_bytes(__import__("os").urandom(4), "little")))
    _w = lambda a: (lambda t: t.astype(jnp.bfloat16) if jnp.issubdtype(t.dtype, jnp.floating) else t)(jnp.asarray(a))

    def _A_setup():
        B, S, Dm = (1, 2048, 1024)
        H, Dh = (32, 128)
        M, seg = (8, 32)
        seg = min(seg, S)
        S = S // seg * seg
        return {'x': _w((lambda *s: _rng.normal(s) * 0.05)(B, S, Dm)), 'mem0': _w((lambda *s: _rng.normal(s) * 0.05)(B, M, Dm)), 'Wq': _w((lambda *s: _rng.normal(s) * 0.05)(Dm, H, Dh) * Dm ** (-0.5)), 'Wk': _w((lambda *s: _rng.normal(s) * 0.05)(Dm, H, Dh) * Dm ** (-0.5)), 'Wv': _w((lambda *s: _rng.normal(s) * 0.05)(Dm, H, Dh) * Dm ** (-0.5)), 'Wo': _w((lambda *s: _rng.normal(s) * 0.05)(H, Dh, Dm) * (H * Dh) ** (-0.5)), 'seg_len': seg}
    _A_in = _A_setup()

    def _B_setup():
        B, S, D, F = (1, 2048, 1024, 3584)
        return {'x': _w((lambda *s: _rng.normal(s) * 0.05)(B, S, D)), 'w_gate': _w((lambda *s: _rng.normal(s) * 0.05)(D, F)), 'w_up': _w((lambda *s: _rng.normal(s) * 0.05)(D, F)), 'w_down': _w((lambda *s: _rng.normal(s) * 0.05)(F, D))}
    _B_in = _B_setup()
    return {'A_x': _A_in['x'], 'A_mem0': _A_in['mem0'], 'A_Wq': _A_in['Wq'], 'A_Wk': _A_in['Wk'], 'A_Wv': _A_in['Wv'], 'A_Wo': _A_in['Wo'], 'A_seg_len': _A_in['seg_len'], 'B_x': _B_in['x'], 'B_w_gate': _B_in['w_gate'], 'B_w_up': _B_in['w_up'], 'B_w_down': _B_in['w_down']}

def reference(A_x, A_mem0, A_Wq, A_Wk, A_Wv, A_Wo, A_seg_len, B_x, B_w_gate, B_w_up, B_w_down):

    def _A_ref(x, mem0, Wq, Wk, Wv, Wo, seg_len):
        B, S, Dm = x.shape
        H, Dh = (Wq.shape[1], Wq.shape[2])
        M = mem0.shape[1]
        scale = Dh ** (-0.5)
        n_seg = S // seg_len
        L = M + seg_len
        idx = jnp.arange(L)
        mask = (idx[:, None] < M) | (idx[:, None] >= idx[None, :])
        mem = mem0
        outs = []
        for s in range(n_seg):
            xs = x[:, s * seg_len:(s + 1) * seg_len, :].copy()
            h = jnp.concatenate([mem, xs], axis=1)
            q = jnp.einsum('btd,dhe->bhte', h, Wq)
            k = jnp.einsum('btd,dhe->bhte', h, Wk)
            v = jnp.einsum('btd,dhe->bhte', h, Wv)
            scores = jnp.einsum('bhqe,bhke->bhqk', q, k) * scale
            scores = jnp.where(mask[None, None], scores, -1000000000.0)
            p = _softmax(scores, axis=-1)
            o = jnp.einsum('bhqk,bhke->bhqe', p, v)
            o = jnp.einsum('bhte,hed->btd', o, Wo)
            mem = o[:, :M, :].copy()
            outs.append(o[:, M:, :])
        return jnp.concatenate(outs, axis=1)

    def _B_ref(x, w_gate, w_up, w_down):
        g = jnp.einsum('bsd,df->bsf', x, w_gate)
        u = jnp.einsum('bsd,df->bsf', x, w_up)
        h = _sigmoid(g) * u
        return jnp.einsum('bsf,fd->bsd', h, w_down)
    x = A_x
    xn = _layernorm(x, axis=-1)
    s = _A_ref(xn, A_mem0, A_Wq, A_Wk, A_Wv, A_Wo, A_seg_len)
    g = _silu(_B_ref(xn, B_w_gate, B_w_up, B_w_down))
    return x + s * g
```

```python
import functools
import jax, jax.numpy as jnp, numpy as np
from jax.experimental import pallas as pl
from jax.experimental.pallas import tpu as pltpu

S, D, H, DH, M, SEG, F = 2048, 1024, 32, 128, 8, 32, 3584
L = M + SEG
NSEG = S // SEG
f32, bf16 = jnp.float32, jnp.bfloat16

def mdot(a, b):
    return jax.lax.dot_general(a, b, (((1,), (0,)), ((), ())), preferred_element_type=f32)

def kern(x_hbm, mem0_ref, wq_hbm, wk_hbm, wv_hbm, wo_hbm, wg_hbm, wu_hbm, wd_hbm, out_hbm,
         x_v, xn_v, g_v, out_v, wq_v, wk_v, wv_v, wo_v, wg_v, wu_v, wd_v, o_scr, q_scr, k_scr, v_scr, sems, osem):
    cx = pltpu.make_async_copy(x_hbm, x_v, sems.at[0]); cx.start()
    cg = pltpu.make_async_copy(wg_hbm, wg_v, sems.at[1]); cg.start()
    cu = pltpu.make_async_copy(wu_hbm, wu_v, sems.at[2]); cu.start()
    cd = pltpu.make_async_copy(wd_hbm, wd_v, sems.at[3]); cd.start()
    cq = pltpu.make_async_copy(wq_hbm, wq_v, sems.at[4]); cq.start()
    ck = pltpu.make_async_copy(wk_hbm, wk_v, sems.at[5]); ck.start()
    cv = pltpu.make_async_copy(wv_hbm, wv_v, sems.at[6]); cv.start()
    co = [pltpu.make_async_copy(wo_hbm.at[:, pl.ds(n * 128, 128)], wo_v.at[n], sems.at[7 + n]) for n in range(8)]
    for c in co: c.start()
    cx.wait()
    def ln(i, c):
        r = pl.ds(pl.multiple_of(i * 128, 128), 128)
        x = x_v[r, :].astype(f32)
        m = jnp.mean(x, axis=-1, keepdims=True)
        xc = x - m
        v = jnp.mean(xc * xc, axis=-1, keepdims=True)
        xn_v[r, :] = (xc * jax.lax.rsqrt(v + 1e-5)).astype(bf16)
        return c
    jax.lax.fori_loop(0, S // 128, ln, 0)
    cg.wait(); cu.wait(); cd.wait()
    RB = 256
    FC = 512
    def ffn(i, c):
        r = pl.ds(pl.multiple_of(i * RB, RB), RB)
        xn = xn_v[r, :]
        acc = jnp.zeros((RB, D), f32)
        for j in range(F // FC):
            g = mdot(xn, wg_v[:, j * FC:(j + 1) * FC])
            u = mdot(xn, wu_v[:, j * FC:(j + 1) * FC])
            h = (jax.nn.sigmoid(g) * u).astype(bf16)
            acc = acc + mdot(h, wd_v[j * FC:(j + 1) * FC, :])
        g_v[r, :] = acc * jax.nn.sigmoid(acc)
        return c
    jax.lax.fori_loop(0, S // RB, ffn, 0)
    cq.wait(); ck.wait(); cv.wait()
    for c in co: c.wait()
    ri = jax.lax.broadcasted_iota(jnp.int32, (L, L), 0)
    ci = jax.lax.broadcasted_iota(jnp.int32, (L, L), 1)
    mask = (ri < M) | (ri >= ci)
    scale = DH ** -0.5
    def step(s, mem):
        r = pl.ds(pl.multiple_of(s * SEG, SEG), SEG)
        hh = jnp.concatenate([mem, xn_v[r, :].astype(f32)], axis=0)
        st = {}
        for h in range(H):
            q_scr[h] = mdot(hh, wq_v[h])
            k_scr[h] = mdot(hh, wk_v[h])
            v_scr[h] = mdot(hh, wv_v[h])
        def s_qk(h):
            sc = jax.lax.dot_general(q_scr[h], k_scr[h].astype(bf16), (((1,), (1,)), ((), ())), preferred_element_type=f32) * scale
            sc = jnp.where(mask, sc, -1e9)
            st[h, 's'] = sc
            st[h, 'm'] = jnp.max(sc, axis=-1, keepdims=True)
        def s_exp(h):
            e = jnp.exp(st.pop((h, 's')) - st.pop((h, 'm')))
            st[h, 'l'] = jnp.sum(e, axis=-1, keepdims=True)
            st[h, 'e'] = mdot(e, v_scr[h].astype(bf16))
        def s_pv(h):
            o_scr[h] = st.pop((h, 'e')) * pl.reciprocal(st.pop((h, 'l')), approx=False)
        def ok(h): return 0 <= h < H
        for t in range(H + 4):
            if ok(t): s_qk(t)
            if ok(t - 2): s_exp(t - 2)
            if ok(t - 4): s_pv(t - 4)
        acc = None
        for h in range(H):
            o = o_scr[h]
            t = jnp.concatenate([mdot(o, wo_v[n, h * 128:(h + 1) * 128, :]) for n in range(8)], axis=1)
            acc = t if acc is None else acc + t
        out_v[r, :] = (x_v[r, :].astype(f32) + acc[M:, :] * g_v[r, :]).astype(bf16)
        return acc[:M, :]
    jax.lax.fori_loop(0, NSEG, step, mem0_ref[...].astype(f32))
    c = pltpu.make_async_copy(out_v, out_hbm, osem); c.start(); c.wait()

@functools.partial(jax.jit, static_argnames=("A_seg_len",))
def pallas_recurrent_scan__memory_aug_recurrent_mem_tr__glu_gated_glu__prompt_kernel(A_x, A_mem0, A_Wq, A_Wk, A_Wv, A_Wo, A_seg_len, B_x, B_w_gate, B_w_up, B_w_down):
    assert A_seg_len == SEG
    x = A_x.reshape(S, D)
    mem0 = A_mem0.reshape(M, D)
    wq = jnp.transpose(A_Wq, (1, 0, 2)); wk = jnp.transpose(A_Wk, (1, 0, 2)); wv = jnp.transpose(A_Wv, (1, 0, 2))
    wo = A_Wo.reshape(H * DH, D)
    anyspec = pl.BlockSpec(memory_space=pl.ANY)
    out = pl.pallas_call(
        kern,
        out_shape=jax.ShapeDtypeStruct((S, D), bf16),
        in_specs=[anyspec, pl.BlockSpec(memory_space=pltpu.VMEM)] + [anyspec] * 7,
        out_specs=anyspec,
        scratch_shapes=[
            pltpu.VMEM((S, D), bf16), pltpu.VMEM((S, D), bf16), pltpu.VMEM((S, D), f32), pltpu.VMEM((S, D), bf16),
            pltpu.VMEM((H, D, DH), bf16), pltpu.VMEM((H, D, DH), bf16), pltpu.VMEM((H, D, DH), bf16),
            pltpu.VMEM((8, H * DH, 128), bf16),
            pltpu.VMEM((D, F), bf16), pltpu.VMEM((D, F), bf16), pltpu.VMEM((F, D), bf16),
            pltpu.VMEM((H, L, DH), f32),pltpu.VMEM((H, L, DH), f32),pltpu.VMEM((H, L, DH), f32),pltpu.VMEM((H, L, DH), f32),
            pltpu.SemaphoreType.DMA((15,)), pltpu.SemaphoreType.DMA,
        ],
        compiler_params=pltpu.CompilerParams(vmem_limit_bytes=110 * 1024 * 1024),
    )(x, mem0, wq, wk, wv, wo, B_w_gate, B_w_up, B_w_down)
    return out.reshape(1, S, D)
```

```python
import functools
import jax, jax.numpy as jnp, numpy as np
from jax.experimental import pallas as pl
from jax.experimental.pallas import tpu as pltpu

S, D, H, DH, M, SEG, F = 2048, 1024, 32, 128, 8, 32, 3584
L = M + SEG
NSEG = S // SEG
f32, bf16, u32 = jnp.float32, jnp.bfloat16, jnp.uint32
RB = 256
FC = 512
NFC = F // FC
FT = FC // 128

def mdot(a, b):
    return jax.lax.dot_general(a, b, (((1,), (0,)), ((), ())), preferred_element_type=f32)

def tobf(w32):
    return pltpu.bitcast(w32, bf16)

def kern(x_hbm, mem0_ref, wq_hbm, wk_hbm, wv_hbm, wo_hbm, wg_hbm, wu_hbm, wd_hbm, out_hbm,
         x_v, xn_v, g_v, out_v, wq_v, wk_v, wv_v, wo_v, wg_v, wu_v, wd_v, raw_v, o_scr, q_scr, k_scr, v_scr,
         xsem, fsem, wsem, osem):
    wo32, wg32, wu32, wd32 = (w.bitcast(u32) for w in (wo_v, wg_v, wu_v, wd_v))
    cx = [pltpu.make_async_copy(x_hbm.at[pl.ds(i * 512, 512)], x_v.at[pl.ds(i * 512, 512)], xsem.at[i]) for i in range(4)]
    def c_gu(j):
        cs = []
        for t in range(FT):
            n = j * FT + t
            cs.append(pltpu.make_async_copy(wg_hbm.at[:, pl.ds(n * 128, 128)], wg_v.at[n], fsem.at[0, j]))
            cs.append(pltpu.make_async_copy(wu_hbm.at[:, pl.ds(n * 128, 128)], wu_v.at[n], fsem.at[1, j]))
        return cs
    def c_d(j):
        return [pltpu.make_async_copy(wd_hbm.at[pl.ds(j * FC, FC), pl.ds(n * 128, 128)], wd_v.at[n, pl.ds(j * FC, FC)], fsem.at[2, j]) for n in range(8)]
    def c_raw():
        return [pltpu.make_async_copy(w.bitcast(u32).at[:, g], raw_v.at[i, g].reshape(D, 8, DH), wsem.at[2 * i + g])
                for i, w in enumerate((wq_hbm, wk_hbm, wv_hbm)) for g in range(2)]
    def c_o():
        return [pltpu.make_async_copy(wo_hbm.at[:, pl.ds(n * 128, 128)], wo_v.at[n], wsem.at[6 + n]) for n in range(8)]
    def start(cs):
        for c in cs: c.start()
    def wait(cs):
        for c in cs: c.wait()

    def ln(i, c):
        r = pl.ds(pl.multiple_of(i * 128, 128), 128)
        x = x_v[r, :].astype(f32)
        m = jnp.mean(x, axis=-1, keepdims=True)
        xc = x - m
        v = jnp.mean(xc * xc, axis=-1, keepdims=True)
        xn_v[r, :] = (xc * jax.lax.rsqrt(v + 1e-5)).astype(bf16)
        return c

    def ffn_block(i, first=False):
        r = pl.ds(pl.multiple_of(i * RB, RB), RB)
        xn = xn_v[r, :]
        acc = jnp.zeros((RB, D), f32)
        for j in range(NFC):
            if first:
                if j == 0:
                    start(c_d(0))
                if j + 1 < NFC:
                    start(c_gu(j + 1)); start(c_d(j + 1))
                if j == 2:
                    start(cx[1:])
                wait(c_gu(j))
            g = jnp.concatenate([mdot(xn, tobf(wg32[j * FT + t])) for t in range(FT)], axis=1)
            u = jnp.concatenate([mdot(xn, tobf(wu32[j * FT + t])) for t in range(FT)], axis=1)
            h = (jax.nn.sigmoid(g) * u).astype(bf16)
            if first:
                wait(c_d(j))
            acc = acc + jnp.concatenate([mdot(h, tobf(wd32[n, j * (FC // 2):(j + 1) * (FC // 2), :])) for n in range(8)], axis=1)
        g_v[r, :] = acc * jax.nn.sigmoid(acc)

    def relayout(i, c):
        r0 = pl.ds(pl.multiple_of(i * 64, 64), 64)
        base = pl.multiple_of(i * 1024, 1024)
        for wi, dst in enumerate((wq_v, wk_v, wv_v)):
            for g in range(2):
                src = raw_v.at[wi, g, pl.ds(base, 1024)]
                for jj in range(8):
                    ev = src[pl.ds(jj, 64, stride=16), :]
                    od = src[pl.ds(8 + jj, 64, stride=16), :]
                    dst[16 * g + 2 * jj, r0, :] = (ev & u32(0xFFFF)) | (od << 16)
                    dst[16 * g + 2 * jj + 1, r0, :] = (ev >> 16) | (od & u32(0xFFFF0000))
        return c

    cx[0].start()
    start(c_gu(0))
    cx[0].wait()
    jax.lax.fori_loop(0, 4, ln, 0)
    ffn_block(0, first=True)
    start(c_raw()); start(c_o())
    wait(cx[1:])
    jax.lax.fori_loop(4, S // 128, ln, 0)
    def ffn_a(i, c):
        ffn_block(i)
        return c
    jax.lax.fori_loop(1, 8, ffn_a, 0)
    wait(c_raw())
    jax.lax.fori_loop(0, 8, relayout, 0)
    wait(c_o())
    ri = jax.lax.broadcasted_iota(jnp.int32, (L, L), 0)
    ci = jax.lax.broadcasted_iota(jnp.int32, (L, L), 1)
    mask = (ri < M) | (ri >= ci)
    scale = DH ** -0.5
    def ocopy(s4):
        r = pl.ds(pl.multiple_of(s4 * 128, 128), 128)
        return pltpu.make_async_copy(out_v.at[r], out_hbm.at[r], osem)
    def step(s, mem):
        r = pl.ds(pl.multiple_of(s * SEG, SEG), SEG)
        hh = jnp.concatenate([mem, xn_v[r, :].astype(f32)], axis=0)
        st = {}
        for h in range(H):
            q_scr[h] = mdot(hh, tobf(wq_v[h]))
            k_scr[h] = mdot(hh, tobf(wk_v[h]))
            v_scr[h] = mdot(hh, tobf(wv_v[h]))
        def s_qk(h):
            sc = jax.lax.dot_general(q_scr[h], k_scr[h].astype(bf16), (((1,), (1,)), ((), ())), preferred_element_type=f32) * scale
            sc = jnp.where(mask, sc, -1e9)
            st[h, 's'] = sc
            st[h, 'm'] = jnp.max(sc, axis=-1, keepdims=True)
        def s_exp(h):
            e = jnp.exp(st.pop((h, 's')) - st.pop((h, 'm')))
            st[h, 'l'] = jnp.sum(e, axis=-1, keepdims=True)
            st[h, 'e'] = mdot(e, v_scr[h].astype(bf16))
        def s_pv(h):
            o_scr[h] = st.pop((h, 'e')) * pl.reciprocal(st.pop((h, 'l')), approx=False)
        def ok(h): return 0 <= h < H
        for t in range(H + 4):
            if ok(t): s_qk(t)
            if ok(t - 2): s_exp(t - 2)
            if ok(t - 4): s_pv(t - 4)
        acc = None
        for h in range(H):
            o = o_scr[h]
            t = jnp.concatenate([mdot(o, tobf(wo32[n, h * 64:(h + 1) * 64, :])) for n in range(8)], axis=1)
            acc = t if acc is None else acc + t
        out_v[r, :] = (x_v[r, :].astype(f32) + acc[M:, :] * g_v[r, :]).astype(bf16)
        @pl.when((s & 3) == 3)
        def _():
            ocopy(s >> 2).start()
        return acc[:M, :]
    jax.lax.fori_loop(0, NSEG, step, mem0_ref[...].astype(f32))
    pltpu.make_async_copy(out_v, out_hbm, osem).wait()

@functools.partial(jax.jit, static_argnames=("A_seg_len",))
def pallas_recurrent_scan__memory_aug_recurrent_mem_tr__glu_gated_glu__prompt_kernel(A_x, A_mem0, A_Wq, A_Wk, A_Wv, A_Wo, A_seg_len, B_x, B_w_gate, B_w_up, B_w_down):
    assert A_seg_len == SEG
    x = A_x.reshape(S, D)
    mem0 = A_mem0.reshape(M, D)
    wq = A_Wq.reshape(D, 2, 16, DH); wk = A_Wk.reshape(D, 2, 16, DH); wv = A_Wv.reshape(D, 2, 16, DH)
    wo = A_Wo.reshape(H * DH, D)
    anyspec = pl.BlockSpec(memory_space=pl.ANY)
    out = pl.pallas_call(
        kern,
        out_shape=jax.ShapeDtypeStruct((S, D), bf16),
        in_specs=[anyspec, pl.BlockSpec(memory_space=pltpu.VMEM)] + [anyspec] * 7,
        out_specs=anyspec,
        scratch_shapes=[
            pltpu.VMEM((S, D), bf16), pltpu.VMEM((S, D), bf16), pltpu.VMEM((S, D), f32), pltpu.VMEM((S, D), bf16),
            pltpu.VMEM((H, D // 2, DH), u32), pltpu.VMEM((H, D // 2, DH), u32), pltpu.VMEM((H, D // 2, DH), u32),
            pltpu.VMEM((8, H * DH, 128), bf16),
            pltpu.VMEM((F // 128, D, 128), bf16), pltpu.VMEM((F // 128, D, 128), bf16), pltpu.VMEM((8, F, 128), bf16),
            pltpu.VMEM((3, 2, D * 8, DH), u32),
            pltpu.VMEM((H, L, DH), f32), pltpu.VMEM((H, L, DH), f32), pltpu.VMEM((H, L, DH), f32), pltpu.VMEM((H, L, DH), f32),
            pltpu.SemaphoreType.DMA((4,)), pltpu.SemaphoreType.DMA((3, NFC)), pltpu.SemaphoreType.DMA((14,)), pltpu.SemaphoreType.DMA,
        ],
        compiler_params=pltpu.CompilerParams(vmem_limit_bytes=120 * 1024 * 1024),
    )(x, mem0, wq, wk, wv, wo, B_w_gate, B_w_up, B_w_down)
    return out.reshape(1, S, D)
```

```python
import functools
import jax, jax.numpy as jnp, numpy as np
from jax.experimental import pallas as pl
from jax.experimental.pallas import tpu as pltpu

S, D, H, DH, M, SEG, F = 2048, 1024, 32, 128, 8, 32, 3584
L = M + SEG
NSEG = S // SEG
f32, bf16, u32 = jnp.float32, jnp.bfloat16, jnp.uint32
RB = 256
FC = 896
NFC = F // FC
FT = FC // 128

def mdot(a, b):
    return jax.lax.dot_general(a, b, (((1,), (0,)), ((), ())), preferred_element_type=f32)

def tobf(w32):
    return pltpu.bitcast(w32, bf16)

def kern(x_hbm, mem0_ref, wq_hbm, wk_hbm, wv_hbm, wo_hbm, wg_hbm, wu_hbm, wd_hbm, out_hbm,
         x_v, xn_v, g_v, out_v, wq_v, wk_v, wv_v, wo_v, wg_v, wu_v, wd_v, raw_v, o_scr, q_scr, k_scr, v_scr,
         xsem, fsem, wsem, osem):
    wo32, wg32, wu32, wd32 = (w.bitcast(u32) for w in (wo_v, wg_v, wu_v, wd_v))
    cx = [pltpu.make_async_copy(x_hbm.at[pl.ds(a, n)], x_v.at[pl.ds(a, n)], xsem.at[i]) for i, (a, n) in enumerate(((0, 256), (256, 1792)))]
    def c_gu(j):
        cs = []
        for t in range(FT):
            n = j * FT + t
            cs.append(pltpu.make_async_copy(wg_hbm.at[:, pl.ds(n * 128, 128)], wg_v.at[n], fsem.at[0, j]))
            cs.append(pltpu.make_async_copy(wu_hbm.at[:, pl.ds(n * 128, 128)], wu_v.at[n], fsem.at[1, j]))
        return cs
    def c_d(j):
        return [pltpu.make_async_copy(wd_hbm.at[pl.ds(j * FC, FC), pl.ds(n * 128, 128)], wd_v.at[n, pl.ds(j * FC, FC)], fsem.at[2, j]) for n in range(8)]
    def c_raw():
        return [pltpu.make_async_copy(w.bitcast(u32).at[:, g], raw_v.at[i, g].reshape(D, 8, DH), wsem.at[2 * i + g])
                for i, w in enumerate((wq_hbm, wk_hbm, wv_hbm)) for g in range(2)]
    def c_o():
        return [pltpu.make_async_copy(wo_hbm.at[:, pl.ds(n * 128, 128)], wo_v.at[n], wsem.at[6 + n]) for n in range(8)]
    def start(cs):
        for c in cs: c.start()
    def wait(cs):
        for c in cs: c.wait()

    def ln(i, c):
        r = pl.ds(pl.multiple_of(i * 128, 128), 128)
        x = x_v[r, :].astype(f32)
        m = jnp.mean(x, axis=-1, keepdims=True)
        xc = x - m
        v = jnp.mean(xc * xc, axis=-1, keepdims=True)
        xn_v[r, :] = (xc * jax.lax.rsqrt(v + 1e-5)).astype(bf16)
        return c

    def ffn_block(i, first=False):
        r = pl.ds(pl.multiple_of(i * RB, RB), RB)
        xn = xn_v[r, :]
        acc = jnp.zeros((RB, D), f32)
        for j in range(NFC):
            if first:
                if j == 0:
                    start(c_d(0))
                if j + 1 < NFC:
                    start(c_gu(j + 1)); start(c_d(j + 1))
                if j == 2:
                    start(cx[1:])
                wait(c_gu(j))
            g = jnp.concatenate([mdot(xn, tobf(wg32[j * FT + t])) for t in range(FT)], axis=1)
            u = jnp.concatenate([mdot(xn, tobf(wu32[j * FT + t])) for t in range(FT)], axis=1)
            h = (jax.nn.sigmoid(g) * u).astype(bf16)
            if first:
                wait(c_d(j))
            acc = acc + jnp.concatenate([mdot(h, tobf(wd32[n, j * (FC // 2):(j + 1) * (FC // 2), :])) for n in range(8)], axis=1)
        g_v[r, :] = acc * jax.nn.sigmoid(acc)

    def relayout(i, c):
        r0 = pl.ds(pl.multiple_of(i * 64, 64), 64)
        base = pl.multiple_of(i * 1024, 1024)
        for wi, dst in enumerate((wq_v, wk_v, wv_v)):
            for g in range(2):
                src = raw_v.at[wi, g, pl.ds(base, 1024)]
                for jj in range(8):
                    ev = src[pl.ds(jj, 64, stride=16), :]
                    od = src[pl.ds(8 + jj, 64, stride=16), :]
                    dst[16 * g + 2 * jj, r0, :] = (ev & u32(0xFFFF)) | (od << 16)
                    dst[16 * g + 2 * jj + 1, r0, :] = (ev >> 16) | (od & u32(0xFFFF0000))
        return c

    cx[0].start()
    start(c_gu(0))
    cx[0].wait()
    jax.lax.fori_loop(0, 2, ln, 0)
    ffn_block(0, first=True)
    start(c_raw()); start(c_o())
    wait(cx[1:])
    jax.lax.fori_loop(2, S // 128, ln, 0)
    def ffn_a(i, c):
        ffn_block(i)
        return c
    jax.lax.fori_loop(1, 8, ffn_a, 0)
    wait(c_raw())
    jax.lax.fori_loop(0, 8, relayout, 0)
    wait(c_o())
    ri = jax.lax.broadcasted_iota(jnp.int32, (L, L), 0)
    ci = jax.lax.broadcasted_iota(jnp.int32, (L, L), 1)
    mask = (ri < M) | (ri >= ci)
    scale = DH ** -0.5
    def ocopy(s4):
        r = pl.ds(pl.multiple_of(s4 * 128, 128), 128)
        return pltpu.make_async_copy(out_v.at[r], out_hbm.at[r], osem)
    def step(s, mem):
        r = pl.ds(pl.multiple_of(s * SEG, SEG), SEG)
        hh = jnp.concatenate([mem, xn_v[r, :].astype(f32)], axis=0)
        st = {}
        for h in range(H):
            q_scr[h] = mdot(hh, tobf(wq_v[h]))
            k_scr[h] = mdot(hh, tobf(wk_v[h]))
            v_scr[h] = mdot(hh, tobf(wv_v[h]))
        def s_qk(h):
            sc = jax.lax.dot_general(q_scr[h], k_scr[h].astype(bf16), (((1,), (1,)), ((), ())), preferred_element_type=f32) * (scale * 1.4426950408889634)
            sc = jnp.where(mask, sc, -1e9 * 1.4426950408889634)
            st[h, 's'] = sc
            st[h, 'm'] = jnp.max(sc, axis=-1, keepdims=True)
        def s_exp(h):
            e = jnp.exp2(st.pop((h, 's')) - st.pop((h, 'm')))
            st[h, 'l'] = jnp.sum(e, axis=-1, keepdims=True)
            st[h, 'e'] = mdot(e, v_scr[h].astype(bf16))
        def s_pv(h):
            l = st.pop((h, 'l'))
            r0 = pl.reciprocal(l, approx=True)
            o_scr[h] = st.pop((h, 'e')) * (r0 * (2.0 - l * r0))
        def ok(h): return 0 <= h < H
        for t in range(H + 4):
            if ok(t): s_qk(t)
            if ok(t - 2): s_exp(t - 2)
            if ok(t - 4): s_pv(t - 4)
        acc = None
        for h in range(H):
            o = o_scr[h]
            t = jnp.concatenate([mdot(o, tobf(wo32[n, h * 64:(h + 1) * 64, :])) for n in range(8)], axis=1)
            acc = t if acc is None else acc + t
        out_v[r, :] = (x_v[r, :].astype(f32) + acc[M:, :] * g_v[r, :]).astype(bf16)
        @pl.when((s & 3) == 3)
        def _():
            ocopy(s >> 2).start()
        return acc[:M, :]
    jax.lax.fori_loop(0, NSEG, step, mem0_ref[...].astype(f32))
    pltpu.make_async_copy(out_v, out_hbm, osem).wait()

@functools.partial(jax.jit, static_argnames=("A_seg_len",))
def pallas_recurrent_scan__memory_aug_recurrent_mem_tr__glu_gated_glu__prompt_kernel(A_x, A_mem0, A_Wq, A_Wk, A_Wv, A_Wo, A_seg_len, B_x, B_w_gate, B_w_up, B_w_down):
    assert A_seg_len == SEG
    x = A_x.reshape(S, D)
    mem0 = A_mem0.reshape(M, D)
    wq = A_Wq.reshape(D, 2, 16, DH); wk = A_Wk.reshape(D, 2, 16, DH); wv = A_Wv.reshape(D, 2, 16, DH)
    wo = A_Wo.reshape(H * DH, D)
    anyspec = pl.BlockSpec(memory_space=pl.ANY)
    out = pl.pallas_call(
        kern,
        out_shape=jax.ShapeDtypeStruct((S, D), bf16),
        in_specs=[anyspec, pl.BlockSpec(memory_space=pltpu.VMEM)] + [anyspec] * 7,
        out_specs=anyspec,
        scratch_shapes=[
            pltpu.VMEM((S, D), bf16), pltpu.VMEM((S, D), bf16), pltpu.VMEM((S, D), f32), pltpu.VMEM((S, D), bf16),
            pltpu.VMEM((H, D // 2, DH), u32), pltpu.VMEM((H, D // 2, DH), u32), pltpu.VMEM((H, D // 2, DH), u32),
            pltpu.VMEM((8, H * DH, 128), bf16),
            pltpu.VMEM((F // 128, D, 128), bf16), pltpu.VMEM((F // 128, D, 128), bf16), pltpu.VMEM((8, F, 128), bf16),
            pltpu.VMEM((3, 2, D * 8, DH), u32),
            pltpu.VMEM((H, L, DH), f32), pltpu.VMEM((H, L, DH), f32), pltpu.VMEM((H, L, DH), f32), pltpu.VMEM((H, L, DH), f32),
            pltpu.SemaphoreType.DMA((2,)), pltpu.SemaphoreType.DMA((3, NFC)), pltpu.SemaphoreType.DMA((14,)), pltpu.SemaphoreType.DMA,
        ],
        compiler_params=pltpu.CompilerParams(vmem_limit_bytes=120 * 1024 * 1024),
    )(x, mem0, wq, wk, wv, wo, B_w_gate, B_w_up, B_w_down)
    return out.reshape(1, S, D)
```
